```python
import os as _os
_os.environ.setdefault("JAX_PLATFORMS", "cpu")
import jax
import jax.numpy as jnp

def _softmax(x, axis=-1):
    return jax.nn.softmax(x, axis=axis)
def _gelu(x):
    return jax.nn.gelu(x, approximate=True)
def _silu(x):
    return jax.nn.silu(x)
def _sigmoid(x):
    return jax.nn.sigmoid(x)
def _layernorm(x, axis=-1, eps=1e-5):
    m = jnp.mean(x, axis=axis, keepdims=True)
    v = jnp.var(x, axis=axis, keepdims=True)
    return (x - m) / jnp.sqrt(v + eps)
def _scatter_add(tgt, idx, src, axis=0):
    return tgt.at[idx].add(src)
def _segment_sum(src, seg, n):
    return jax.ops.segment_sum(src, seg, n)
class _Rng:
    def __init__(self, key):
        self._k = key
    def _next(self):
        self._k, sub = jax.random.split(self._k)
        return sub
    def normal(self, shape):
        return jax.random.normal(self._next(), shape, dtype=jnp.bfloat16)
    def randint(self, lo, hi, shape):
        return jax.random.randint(self._next(), shape, lo, hi, dtype=jnp.int32)
    def uniform(self, shape, lo=0.0, hi=1.0):
        return jax.random.uniform(self._next(), shape, jnp.bfloat16, lo, hi)
    def permutation(self, n):
        return jax.random.permutation(self._next(), n)


kernel_name = 'gated_mix__mha_block__mixer_s_mlp__prompt'

def setup_inputs():
    _rng = _Rng(jax.random.key(int.from_bytes(__import__("os").urandom(4), "little")))
    _w = (lambda a: (lambda t: t.astype(jnp.bfloat16) if jnp.issubdtype(t.dtype, jnp.floating) else t)(jnp.asarray(a)))
    def _A_setup():
        B, S, D, H = 1, 2048, 512, 32
        return {
            "x": _w((lambda *s: _rng.normal(s) * 0.05)(B, S, D)),
            "wqkv": _w((lambda *s: _rng.normal(s) * 0.8)(D, 3 * D)),
            "wo": _w((lambda *s: _rng.normal(s) * 0.05)(D, D)),
        }
    _A_in = _A_setup()

    def _B_setup():
        B, S, D, F = 1, 2048, 512, 1792
        return {
            "x":  _w((lambda *s: _rng.normal(s) * 0.05)(B, S, D)),
            "w1": _w((lambda *s: _rng.normal(s) * 0.2)(D, D) * (D ** -0.5)),
            "w2": _w((lambda *s: _rng.normal(s) * 0.2)(D, D) * (D ** -0.5)),
            "w3": _w((lambda *s: _rng.normal(s) * 0.2)(D, F) * (D ** -0.5)),
            "w4": _w((lambda *s: _rng.normal(s) * 0.2)(F, D) * (F ** -0.5)),
        }
    _B_in = _B_setup()

    return {
        "A_x": _A_in["x"],
        "A_wqkv": _A_in["wqkv"],
        "A_wo": _A_in["wo"],
        "B_x": _B_in["x"],
        "B_w1": _B_in["w1"],
        "B_w2": _B_in["w2"],
        "B_w3": _B_in["w3"],
        "B_w4": _B_in["w4"],
        "gate_w": _w((lambda *s: _rng.normal(s) * 0.05)(512) * 16.0),
    }

def reference(A_x, A_wqkv, A_wo, B_x, B_w1, B_w2, B_w3, B_w4, gate_w):
    def _A_ref(x, wqkv, wo):
        B, S, D = x.shape
        H = 32
        Dh = D // H
        qkv = (lambda x, *d: x.transpose(*d))((x @ wqkv).reshape(B, S, 3, H, Dh), 2, 0, 3, 1, 4)
        q, k, v = qkv[0], qkv[1], qkv[2]
        scores = jnp.einsum("bhqd,bhkd->bhqk", q, k) * (Dh ** -0.5)
        p = _softmax(scores, axis=-1)
        o = jnp.einsum("bhqk,bhkd->bhqd", p, v)
        return (lambda x, *d: x.transpose(*d))(o, 0, 2, 1, 3).reshape(B, S, D) @ wo

    def _B_ref(x, w1, w2, w3, w4):
        B, S, D = x.shape
        h = _gelu(_layernorm(x, axis=-1) @ w1)
        c = D // 4
        g0 = jnp.pad(h[:, :, 0*c:1*c], ((0, 0), (1, 0), (0, 0)))[:, :S, :]
        g1 = jnp.pad(h[:, :, 1*c:2*c], ((0, 0), (0, 1), (0, 0)))[:, 1:, :]
        g2 = jnp.pad(h[:, :, 2*c:3*c], ((0, 0), (2, 0), (0, 0)))[:, :S, :]
        g3 = jnp.pad(h[:, :, 3*c:   ], ((0, 0), (0, 2), (0, 0)))[:, 2:, :]
        hs = jnp.concatenate([g0, g1, g2, g3], axis=-1) @ w2
        x1 = x + hs
        h2 = _gelu(_layernorm(x1, axis=-1) @ w3) @ w4
        return x1 + h2

    x = A_x
    g = _sigmoid((x * gate_w).sum(-1, keepdims=True))
    a = _A_ref(x, A_wqkv, A_wo)
    b = _B_ref(x, B_w1, B_w2, B_w3, B_w4)
    return g * a + (1 - g) * b
```

```python
import math

import jax
import jax.numpy as jnp
import jax.experimental.pallas as pl
import jax.experimental.pallas.tpu as pltpu

S = 2048
D = 512
H = 32
DH = 16
F = 1792
LANES = 128
HPG = LANES // DH
PAD = 8

TQ = 512
TK = 128
LA = 2
HU = 8
RB = 256

LOG2E = math.log2(math.e)
QSCALE = (DH ** -0.5) * LOG2E
SAFE_LOG2 = 40.0
SAFE_V = 2.0 ** 60

_F32 = jnp.float32
_BF16 = jnp.bfloat16


def _dot(a, b):
    return jnp.dot(a, b, preferred_element_type=_F32)


def _dot_dims(a, b, ca, cb):
    return jax.lax.dot_general(a, b, (((ca,), (cb,)), ((), ())), preferred_element_type=_F32)


def _layernorm(x):
    m = jnp.mean(x, axis=-1, keepdims=True)
    xc = x - m
    v = jnp.mean(xc * xc, axis=-1, keepdims=True)
    return xc * jax.lax.rsqrt(v + 1e-5)


def _gelu(x):
    c = math.sqrt(2.0 / math.pi)
    return 0.5 * x * (1.0 + jnp.tanh(c * (x + 0.044715 * (x * x * x))))


def _kernel(ax_ref, wqkv_ref, wo_ref, w1_ref, w2_ref, w3_ref, w4_ref, gw_ref,
            out_ref,
            qt_ref, k_ref, vt_ref, ot_ref, h_ref):
    head_of_col = jax.lax.broadcasted_iota(jnp.int32, (D, LANES), 0) // DH
    col = jax.lax.broadcasted_iota(jnp.int32, (D, LANES), 1)
    e_mat = jnp.where(head_of_col == col, 1.0, 0.0).astype(_BF16)
    head_of_row = jax.lax.broadcasted_iota(jnp.int32, (H, D), 1) // DH
    rowi = jax.lax.broadcasted_iota(jnp.int32, (H, D), 0)
    et_mat = jnp.where(head_of_row == rowi, 1.0, 0.0).astype(_BF16)

    PB = 512
    qn = jnp.zeros((H, PB), _F32)
    kn = jnp.zeros((PB, LANES), _F32)
    vmax = jnp.zeros((D, PB), _F32)
    for r in range(S // PB):
        x = ax_ref[pl.ds(r * PB, PB), :]
        kk = _dot(x, wqkv_ref[:, D:2 * D]).astype(_BF16)
        k_ref[pl.ds(r * PB, PB), :] = kk
        kf = kk.astype(_F32)
        kn = jnp.maximum(kn, _dot((kf * kf).astype(_BF16), e_mat))
        qt = (_dot_dims(wqkv_ref[:, 0:D], x, 0, 1) * QSCALE).astype(_BF16)
        qt_ref[:, pl.ds(r * PB, PB)] = qt
        qf = qt.astype(_F32)
        qn = jnp.maximum(qn, _dot(et_mat, (qf * qf).astype(_BF16)))
        vt = _dot_dims(wqkv_ref[:, 2 * D:3 * D], x, 0, 1).astype(_BF16)
        vt_ref[:, pl.ds(r * PB, PB)] = vt
        vmax = jnp.maximum(vmax, jnp.abs(vt.astype(_F32)))
    bound2 = jnp.max(qn) * jnp.max(kn) * 1.02
    safe = jnp.logical_and(bound2 <= SAFE_LOG2 * SAFE_LOG2, jnp.max(vmax) <= SAFE_V)

    nq = S // TQ
    nc = S // TK

    def masked_q(h, q0):
        g0 = pl.multiple_of((h // HPG) * LANES, LANES)
        qg = qt_ref[pl.ds(g0, LANES), pl.ds(q0, TQ)]
        row = jax.lax.broadcasted_iota(jnp.int32, (LANES, TQ), 0) // DH
        return jnp.where(row == (h % HPG), qg, jnp.zeros_like(qg)), g0

    @pl.when(safe)
    def _fast():
        nhg = H // HU

        def body(it, carry):
            qb = it // nhg
            hg = it % nhg
            q0 = pl.multiple_of(qb * TQ, TQ)
            wqs = {}

            def qk(t):
                j, c = divmod(t, nc)
                if j not in wqs:
                    wqs[j] = masked_q(hg * HU + j, q0)
                wq, g0 = wqs[j]
                return _dot(k_ref[pl.ds(c * TK, TK), pl.ds(g0, LANES)], wq)

            total = HU * nc
            ss = {t: qk(t) for t in range(min(LA, total))}
            acc = l = None
            for t in range(total):
                j, c = divmod(t, nc)
                h0 = pl.multiple_of((hg * HU + j) * DH, DH)
                if c == 0:
                    acc = jnp.zeros((DH, TQ), _F32)
                    l = jnp.zeros((8, TQ), _F32)
                if t + LA < total:
                    ss[t + LA] = qk(t + LA)
                p = jnp.exp2(ss.pop(t))
                l = l + jnp.sum(p.reshape(TK // 8, 8, TQ), axis=0)
                acc = acc + _dot(vt_ref[pl.ds(h0, DH), pl.ds(c * TK, TK)], p.astype(_BF16))
                if c == nc - 1:
                    lsum = jnp.sum(l, axis=0, keepdims=True)
                    ot_ref[pl.ds(h0, DH), pl.ds(q0, TQ)] = (acc / lsum).astype(_BF16)
            return carry

        jax.lax.fori_loop(0, nq * nhg, body, 0)

    @pl.when(jnp.logical_not(safe))
    def _slow():
        def body(it, carry):
            qb = it // H
            h = it % H
            q0 = pl.multiple_of(qb * TQ, TQ)
            h0 = pl.multiple_of(h * DH, DH)
            wq, g0 = masked_q(h, q0)
            s = _dot(k_ref[:, pl.ds(g0, LANES)], wq)
            m = jnp.max(s, axis=0, keepdims=True)
            p = jnp.exp2(s - m)
            lsum = jnp.sum(p, axis=0, keepdims=True)
            acc = _dot(vt_ref[pl.ds(h0, DH), :], p.astype(_BF16))
            ot_ref[pl.ds(h0, DH), pl.ds(q0, TQ)] = (acc / lsum).astype(_BF16)
            return carry

        jax.lax.fori_loop(0, nq * H, body, 0)

    h_ref[pl.ds(0, PAD), :] = jnp.zeros((PAD, D), _F32)
    h_ref[pl.ds(PAD + S, PAD), :] = jnp.zeros((PAD, D), _F32)
    for r in range(S // RB):
        xb = ax_ref[pl.ds(r * RB, RB), :].astype(_F32)
        hh = _gelu(_dot(_layernorm(xb).astype(_BF16), w1_ref[...]))
        h_ref[pl.ds(PAD + r * RB, RB), :] = hh

    shifts = (-1, 1, -2, 2)
    for r in range(S // RB):
        r0 = r * RB
        hs_in = jnp.concatenate(
            [h_ref[pl.ds(PAD + r0 + shifts[j], RB), pl.ds(j * LANES, LANES)] for j in range(4)],
            axis=-1).astype(_BF16)
        xa = ax_ref[pl.ds(r0, RB), :].astype(_F32)
        x1 = xa + _dot(hs_in, w2_ref[...])
        h2 = _gelu(_dot(_layernorm(x1).astype(_BF16), w3_ref[...])).astype(_BF16)
        b = x1 + _dot(h2, w4_ref[...])
        a = _dot_dims(ot_ref[:, pl.ds(r0, RB)], wo_ref[...], 0, 0)
        g = jax.nn.sigmoid(jnp.sum(xa * gw_ref[...].astype(_F32), axis=-1, keepdims=True))
        out_ref[pl.ds(r0, RB), :] = (g * a + (1.0 - g) * b).astype(out_ref.dtype)


@jax.jit
def pallas_gated_mix__mha_block__mixer_s_mlp__prompt_kernel(
    A_x: jax.Array,
    A_wqkv: jax.Array,
    A_wo: jax.Array,
    B_x: jax.Array,
    B_w1: jax.Array,
    B_w2: jax.Array,
    B_w3: jax.Array,
    B_w4: jax.Array,
    gate_w: jax.Array,
):
    ax = A_x.reshape(S, D)
    gw = gate_w.reshape(1, D)
    out = pl.pallas_call(
        _kernel,
        out_shape=jax.ShapeDtypeStruct((S, D), A_x.dtype),
        scratch_shapes=[
            pltpu.VMEM((D, S), _BF16),
            pltpu.VMEM((S, D), _BF16),
            pltpu.VMEM((D, S), _BF16),
            pltpu.VMEM((D, S), _BF16),
            pltpu.VMEM((S + 2 * PAD, D), _F32),
        ],
        compiler_params=pltpu.CompilerParams(vmem_limit_bytes=100 * 1024 * 1024),
    )(ax, A_wqkv, A_wo, B_w1, B_w2, B_w3, B_w4, gw)
    return out.reshape(1, S, D)
```

```python
import math

import jax
import jax.numpy as jnp
import jax.experimental.pallas as pl
import jax.experimental.pallas.tpu as pltpu

S = 2048
D = 512
H = 32
DH = 16
F = 1792
LANES = 128
HPG = LANES // DH
PAD = 8

TQ = 512
TK = 128
LA = 2
HU = 8
RB = 256
PB = 512

LOG2E = math.log2(math.e)
QSCALE = (DH ** -0.5) * LOG2E
SAFE_LOG2 = 40.0
SAFE_V = 2.0 ** 60

_F32 = jnp.float32
_BF16 = jnp.bfloat16


def _dot(a, b):
    return jnp.dot(a, b, preferred_element_type=_F32)


def _dot_dims(a, b, ca, cb):
    return jax.lax.dot_general(a, b, (((ca,), (cb,)), ((), ())), preferred_element_type=_F32)


def _layernorm(x):
    m = jnp.mean(x, axis=-1, keepdims=True)
    xc = x - m
    v = jnp.mean(xc * xc, axis=-1, keepdims=True)
    return xc * jax.lax.rsqrt(v + 1e-5)


def _gelu(x):
    c = math.sqrt(2.0 / math.pi)
    return 0.5 * x * (1.0 + jnp.tanh(c * (x + 0.044715 * (x * x * x))))


def _kernel(x_hbm, wqkv_hbm, wo_hbm, w1_hbm, w2_hbm, w3_hbm, w4_hbm, gw_ref,
            out_hbm,
            x_ref, wqkv_ref, wo_ref, w1_ref, w2_ref, w3_ref, w4_ref,
            qt_ref, k_ref, vt_ref, ot_ref, h_ref, b_ref, o_stage, in_sems, out_sems):
    copies = {}
    order = []
    def add(name, src, dst):
        copies[name] = pltpu.make_async_copy(src, dst, in_sems.at[len(order)])
        order.append(name)
    add("x0", x_hbm.at[pl.ds(0, PB), :], x_ref.at[pl.ds(0, PB), :])
    add("wk", wqkv_hbm.at[:, pl.ds(D, D)], wqkv_ref.at[:, pl.ds(D, D)])
    add("wq", wqkv_hbm.at[:, pl.ds(0, D)], wqkv_ref.at[:, pl.ds(0, D)])
    add("wv", wqkv_hbm.at[:, pl.ds(2 * D, D)], wqkv_ref.at[:, pl.ds(2 * D, D)])
    for r in range(1, S // PB):
        add(f"x{r}", x_hbm.at[pl.ds(r * PB, PB), :], x_ref.at[pl.ds(r * PB, PB), :])
    add("w1", w1_hbm, w1_ref)
    add("w2", w2_hbm, w2_ref)
    add("w3", w3_hbm, w3_ref)
    add("w4", w4_hbm, w4_ref)
    add("wo", wo_hbm, wo_ref)
    for name in order:
        copies[name].start()

    head_of_col = jax.lax.broadcasted_iota(jnp.int32, (H, D), 1) // DH
    rowi = jax.lax.broadcasted_iota(jnp.int32, (H, D), 0)
    et_mat = jnp.where(head_of_col == rowi, 1.0, 0.0).astype(_BF16)

    qn = jnp.zeros((H, PB), _F32)
    kn = jnp.zeros((H, PB), _F32)
    vmax = jnp.zeros((D, PB), _F32)
    for r in range(S // PB):
        copies[f"x{r}"].wait()
        x = x_ref[pl.ds(r * PB, PB), :]
        if r == 0:
            copies["wk"].wait()
        kk = _dot(x, wqkv_ref[:, D:2 * D]).astype(_BF16)
        k_ref[pl.ds(r * PB, PB), :] = kk
        kf = kk.astype(_F32)
        kn = jnp.maximum(kn, _dot_dims(et_mat, (kf * kf).astype(_BF16), 1, 1))
        if r == 0:
            copies["wq"].wait()
        qt = (_dot_dims(wqkv_ref[:, 0:D], x, 0, 1) * QSCALE).astype(_BF16)
        qt_ref[:, pl.ds(r * PB, PB)] = qt
        qf = qt.astype(_F32)
        qn = jnp.maximum(qn, _dot(et_mat, (qf * qf).astype(_BF16)))
        if r == 0:
            copies["wv"].wait()
        vt = _dot_dims(wqkv_ref[:, 2 * D:3 * D], x, 0, 1).astype(_BF16)
        vt_ref[:, pl.ds(r * PB, PB)] = vt
        vmax = jnp.maximum(vmax, jnp.abs(vt.astype(_F32)))
    bound2 = jnp.max(qn) * jnp.max(kn) * 1.02
    safe = jnp.logical_and(bound2 <= SAFE_LOG2 * SAFE_LOG2, jnp.max(vmax) <= SAFE_V)

    copies["w1"].wait()
    h_ref[pl.ds(0, PAD), :] = jnp.zeros((PAD, D), _F32)
    h_ref[pl.ds(PAD + S, PAD), :] = jnp.zeros((PAD, D), _F32)
    for r in range(S // RB):
        xb = x_ref[pl.ds(r * RB, RB), :].astype(_F32)
        hh = _gelu(_dot(_layernorm(xb).astype(_BF16), w1_ref[...]))
        h_ref[pl.ds(PAD + r * RB, RB), :] = hh

    copies["w2"].wait()
    copies["w3"].wait()
    copies["w4"].wait()
    copies["wo"].wait()
    shifts = (-1, 1, -2, 2)
    for r in range(S // RB):
        r0 = r * RB
        hs_in = jnp.concatenate(
            [h_ref[pl.ds(PAD + r0 + shifts[j], RB), pl.ds(j * LANES, LANES)] for j in range(4)],
            axis=-1).astype(_BF16)
        x1 = x_ref[pl.ds(r0, RB), :].astype(_F32) + _dot(hs_in, w2_ref[...])
        h2 = _gelu(_dot(_layernorm(x1).astype(_BF16), w3_ref[...])).astype(_BF16)
        b_ref[pl.ds(r0, RB), :] = x1 + _dot(h2, w4_ref[...])

    nq = S // TQ
    nc = S // TK

    def masked_q(h, q0):
        g0 = pl.multiple_of((h // HPG) * LANES, LANES)
        qg = qt_ref[pl.ds(g0, LANES), pl.ds(q0, TQ)]
        row = jax.lax.broadcasted_iota(jnp.int32, (LANES, TQ), 0) // DH
        return jnp.where(row == (h % HPG), qg, jnp.zeros_like(qg)), g0

    def out_copy(qb):
        q0 = qb * TQ
        return pltpu.make_async_copy(o_stage.at[pl.ds(q0, TQ), :], out_hbm.at[pl.ds(q0, TQ), :], out_sems.at[qb])

    def finalize(qb):
        for r in range(TQ // RB):
            r0 = qb * TQ + r * RB
            a = _dot_dims(ot_ref[:, pl.ds(r0, RB)], wo_ref[...], 0, 0)
            xa = x_ref[pl.ds(r0, RB), :].astype(_F32)
            g = jax.nn.sigmoid(jnp.sum(xa * gw_ref[...].astype(_F32), axis=-1, keepdims=True))
            o_stage[pl.ds(r0, RB), :] = (g * a + (1.0 - g) * b_ref[pl.ds(r0, RB), :]).astype(o_stage.dtype)
        out_copy(qb).start()

    nhg = H // HU
    for qb in range(nq):
        q0 = qb * TQ

        @pl.when(safe)
        def _fast():
            def body(hg, carry):
                wqs = {}

                def qk(t):
                    j, c = divmod(t, nc)
                    if j not in wqs:
                        wqs[j] = masked_q(hg * HU + j, q0)
                    wq, g0 = wqs[j]
                    return _dot(k_ref[pl.ds(c * TK, TK), pl.ds(g0, LANES)], wq)

                total = HU * nc
                ss = {t: qk(t) for t in range(min(LA, total))}
                acc = l = None
                for t in range(total):
                    j, c = divmod(t, nc)
                    h0 = pl.multiple_of((hg * HU + j) * DH, DH)
                    if c == 0:
                        acc = jnp.zeros((DH, TQ), _F32)
                        l = jnp.zeros((8, TQ), _F32)
                    if t + LA < total:
                        ss[t + LA] = qk(t + LA)
                    p = jnp.exp2(ss.pop(t))
                    l = l + jnp.sum(p.reshape(TK // 8, 8, TQ), axis=0)
                    acc = acc + _dot(vt_ref[pl.ds(h0, DH), pl.ds(c * TK, TK)], p.astype(_BF16))
                    if c == nc - 1:
                        lsum = jnp.sum(l, axis=0, keepdims=True)
                        ot_ref[pl.ds(h0, DH), pl.ds(q0, TQ)] = (acc / lsum).astype(_BF16)
                return carry

            jax.lax.fori_loop(0, nhg, body, 0)

        @pl.when(jnp.logical_not(safe))
        def _slow():
            def body(h, carry):
                h0 = pl.multiple_of(h * DH, DH)
                wq, g0 = masked_q(h, q0)
                s = _dot(k_ref[:, pl.ds(g0, LANES)], wq)
                m = jnp.max(s, axis=0, keepdims=True)
                p = jnp.exp2(s - m)
                lsum = jnp.sum(p, axis=0, keepdims=True)
                acc = _dot(vt_ref[pl.ds(h0, DH), :], p.astype(_BF16))
                ot_ref[pl.ds(h0, DH), pl.ds(q0, TQ)] = (acc / lsum).astype(_BF16)
                return carry

            jax.lax.fori_loop(0, H, body, 0)

        finalize(qb)

    for qb in range(nq):
        out_copy(qb).wait()


@jax.jit
def pallas_gated_mix__mha_block__mixer_s_mlp__prompt_kernel(
    A_x: jax.Array,
    A_wqkv: jax.Array,
    A_wo: jax.Array,
    B_x: jax.Array,
    B_w1: jax.Array,
    B_w2: jax.Array,
    B_w3: jax.Array,
    B_w4: jax.Array,
    gate_w: jax.Array,
):
    ax = A_x.reshape(S, D)
    gw = gate_w.reshape(1, D)
    hbm = pl.BlockSpec(memory_space=pl.ANY)
    out = pl.pallas_call(
        _kernel,
        out_shape=jax.ShapeDtypeStruct((S, D), A_x.dtype),
        in_specs=[hbm] * 7 + [pl.BlockSpec(memory_space=pltpu.VMEM)],
        out_specs=hbm,
        scratch_shapes=[
            pltpu.VMEM((S, D), _BF16),
            pltpu.VMEM((D, 3 * D), _BF16),
            pltpu.VMEM((D, D), _BF16),
            pltpu.VMEM((D, D), _BF16),
            pltpu.VMEM((D, D), _BF16),
            pltpu.VMEM((D, F), _BF16),
            pltpu.VMEM((F, D), _BF16),
            pltpu.VMEM((D, S), _BF16),
            pltpu.VMEM((S, D), _BF16),
            pltpu.VMEM((D, S), _BF16),
            pltpu.VMEM((D, S), _BF16),
            pltpu.VMEM((S + 2 * PAD, D), _F32),
            pltpu.VMEM((S, D), _F32),
            pltpu.VMEM((S, D), _BF16),
            pltpu.SemaphoreType.DMA((12,)),
            pltpu.SemaphoreType.DMA((S // TQ,)),
        ],
        compiler_params=pltpu.CompilerParams(vmem_limit_bytes=100 * 1024 * 1024),
    )(ax, A_wqkv, A_wo, B_w1, B_w2, B_w3, B_w4, gw)
    return out.reshape(1, S, D)
```

```python
import math

import jax
import jax.numpy as jnp
import jax.experimental.pallas as pl
import jax.experimental.pallas.tpu as pltpu

S = 2048
D = 512
H = 32
DH = 16
F = 1792
LANES = 128
HPG = LANES // DH
PAD = 8

TQ = 512
TK = 128
LA = 2
HU = 8
RB = 256
NRB = S // RB

LOG2E = math.log2(math.e)
QSCALE = (DH ** -0.5) * LOG2E
SAFE_LOG2 = 40.0
SAFE_V = 2.0 ** 60

_F32 = jnp.float32
_BF16 = jnp.bfloat16


def _dot(a, b):
    return jnp.dot(a, b, preferred_element_type=_F32)


def _dot_dims(a, b, ca, cb):
    return jax.lax.dot_general(a, b, (((ca,), (cb,)), ((), ())), preferred_element_type=_F32)


def _layernorm(x):
    m = jnp.mean(x, axis=-1, keepdims=True)
    xc = x - m
    v = jnp.mean(xc * xc, axis=-1, keepdims=True)
    return xc * jax.lax.rsqrt(v + 1e-5)


def _gelu(x):
    c = math.sqrt(2.0 / math.pi)
    return 0.5 * x * (1.0 + jnp.tanh(c * (x + 0.044715 * (x * x * x))))


def _mult(v, m):
    return v if isinstance(v, int) else pl.multiple_of(v, m)


def _kernel(x_hbm, wqkv_hbm, wo_hbm, w1_hbm, w2_hbm, w3_hbm, w4_hbm, gw_hbm,
            out_hbm,
            x_ref, wqkv_ref, wo_ref, w1_ref, w2_ref, w3_ref, w4_ref, gw_ref,
            qt_ref, k_ref, vt_ref, ot_ref, h_ref, b_ref, o_stage, nrm_ref, wqvt_ref, spre_ref,
            x_sems, w_sems, out_sems):
    def x_copy(r):
        r0 = _mult(r * RB, RB)
        return pltpu.make_async_copy(x_hbm.at[pl.ds(r0, RB), :], x_ref.at[pl.ds(r0, RB), :], x_sems.at[r])

    w_copies = {
        "wk": pltpu.make_async_copy(wqkv_hbm.at[:, pl.ds(D, D)], wqkv_ref.at[:, pl.ds(D, D)], w_sems.at[0]),
        "wq": pltpu.make_async_copy(wqkv_hbm.at[:, pl.ds(0, D)], wqkv_ref.at[:, pl.ds(0, D)], w_sems.at[1]),
        "wv": pltpu.make_async_copy(wqkv_hbm.at[:, pl.ds(2 * D, D)], wqkv_ref.at[:, pl.ds(2 * D, D)], w_sems.at[2]),
        "w1": pltpu.make_async_copy(w1_hbm, w1_ref, w_sems.at[3]),
        "w2": pltpu.make_async_copy(w2_hbm, w2_ref, w_sems.at[4]),
        "w3": pltpu.make_async_copy(w3_hbm, w3_ref, w_sems.at[5]),
        "w4": pltpu.make_async_copy(w4_hbm, w4_ref, w_sems.at[6]),
        "wo": pltpu.make_async_copy(wo_hbm, wo_ref, w_sems.at[7]),
        "gw": pltpu.make_async_copy(gw_hbm, gw_ref, w_sems.at[8]),
    }
    x_copy(0).start()
    for name in ("wk", "w1", "wq", "wv"):
        w_copies[name].start()
    for r in range(1, NRB):
        x_copy(r).start()
    for name in ("w2", "w3", "w4", "wo", "gw"):
        w_copies[name].start()

    head_of_col = jax.lax.broadcasted_iota(jnp.int32, (H, D), 1) // DH
    rowi = jax.lax.broadcasted_iota(jnp.int32, (H, D), 0)

    h_ref[pl.ds(0, PAD), :] = jnp.zeros((PAD, D), _F32)
    h_ref[pl.ds(PAD + S, PAD), :] = jnp.zeros((PAD, D), _F32)
    nrm_ref[...] = jnp.zeros(nrm_ref.shape, _F32)

    def proj(r, first):
        r0 = _mult(r * RB, RB)
        et_mat = jnp.where(head_of_col == rowi, 1.0, 0.0).astype(_BF16)
        x_copy(r).wait()
        x = x_ref[pl.ds(r0, RB), :]
        if first:
            w_copies["wk"].wait()
        kk = _dot(x, wqkv_ref[:, D:2 * D]).astype(_BF16)
        k_ref[pl.ds(r0, RB), :] = kk
        kf = kk.astype(_F32)
        kn = _dot_dims(et_mat, (kf * kf).astype(_BF16), 1, 1)
        if first:
            w_copies["w1"].wait()
        hh = _gelu(_dot(_layernorm(x.astype(_F32)).astype(_BF16), w1_ref[...]))
        h_ref[pl.ds(_mult(PAD + r0, 8), RB), :] = hh
        if first:
            w_copies["wq"].wait()
            w_copies["wv"].wait()
            wqvt_ref[pl.ds(0, D), :] = wqkv_ref[:, 0:D].T
            wqvt_ref[pl.ds(D, D), :] = wqkv_ref[:, 2 * D:3 * D].T
        qvt = _dot_dims(wqvt_ref[...], x, 1, 1)
        qt = (qvt[:D] * QSCALE).astype(_BF16)
        qt_ref[:, pl.ds(r0, RB)] = qt
        qf = qt.astype(_F32)
        qn = _dot(et_mat, (qf * qf).astype(_BF16))
        vt = qvt[D:].astype(_BF16)
        vt_ref[:, pl.ds(r0, RB)] = vt
        va = jnp.abs(vt.astype(_F32))
        vm = jnp.max(va.reshape(D // H, H, RB), axis=0)
        nrm_ref[0] = jnp.maximum(nrm_ref[0], qn)
        nrm_ref[1] = jnp.maximum(nrm_ref[1], kn)
        nrm_ref[2] = jnp.maximum(nrm_ref[2], vm)

    proj(0, True)

    def proj_body(r, c):
        proj(r, False)
        return c
    jax.lax.fori_loop(1, NRB, proj_body, 0)

    bound2 = jnp.max(nrm_ref[0]) * jnp.max(nrm_ref[1]) * 1.02
    safe = jnp.logical_and(bound2 <= SAFE_LOG2 * SAFE_LOG2, jnp.max(nrm_ref[2]) <= SAFE_V)

    for name in ("w2", "w3", "w4", "wo", "gw"):
        w_copies[name].wait()
    shifts = (-1, 1, -2, 2)

    def mlp_body(i, c):
        r0s = [pl.multiple_of((2 * i + u) * RB, RB) for u in range(2)]
        x1s = []
        for r0 in r0s:
            win = [h_ref[pl.ds(r0, RB + 2 * PAD), pl.ds(j * LANES, LANES)] for j in range(4)]
            hs_in = jnp.concatenate(
                [win[j][PAD + shifts[j]:PAD + shifts[j] + RB] for j in range(4)], axis=-1).astype(_BF16)
            x1s.append(x_ref[pl.ds(r0, RB), :].astype(_F32) + _dot(hs_in, w2_ref[...]))
        h2s = [_gelu(_dot(_layernorm(x1).astype(_BF16), w3_ref[...])).astype(_BF16) for x1 in x1s]
        for r0, x1, h2 in zip(r0s, x1s, h2s):
            b_ref[pl.ds(r0, RB), :] = x1 + _dot(h2, w4_ref[...])
        return c
    jax.lax.fori_loop(0, NRB // 2, mlp_body, 0)

    nq = S // TQ
    nc = S // TK

    def masked_q(h, q0):
        g0 = _mult((h // HPG) * LANES, LANES)
        qg = qt_ref[pl.ds(g0, LANES), pl.ds(q0, TQ)]
        row = jax.lax.broadcasted_iota(jnp.int32, (LANES, TQ), 0) // DH
        return jnp.where(row == (h % HPG), qg, jnp.zeros_like(qg)), g0

    def out_copy(qb):
        q0 = _mult(qb * TQ, TQ)
        return pltpu.make_async_copy(o_stage.at[pl.ds(q0, TQ), :], out_hbm.at[pl.ds(q0, TQ), :], out_sems.at[qb])

    def finalize(qb):
        for r in range(TQ // RB):
            r0 = pl.multiple_of(qb * TQ + r * RB, RB)
            a = _dot_dims(ot_ref[:, pl.ds(r0, RB)], wo_ref[...], 0, 0)
            xa = x_ref[pl.ds(r0, RB), :].astype(_F32)
            g = jax.nn.sigmoid(jnp.sum(xa * gw_ref[...].astype(_F32).reshape(1, D), axis=-1, keepdims=True))
            o_stage[pl.ds(r0, RB), :] = (g * a + (1.0 - g) * b_ref[pl.ds(r0, RB), :]).astype(o_stage.dtype)
        out_copy(qb).start()

    nhg = H // HU

    def prefetch_qk(hg, q0):
        wq, g0 = masked_q(hg * HU, q0)
        return [_dot(k_ref[pl.ds(c * TK, TK), pl.ds(g0, LANES)], wq) for c in range(LA)]

    def fast_heads(hg, q0, hg_n, q0_n):
        wqs = {}

        def qk(t):
            j, c = divmod(t, nc)
            if j not in wqs:
                wqs[j] = masked_q(hg * HU + j, q0)
            wq, g0 = wqs[j]
            return _dot(k_ref[pl.ds(c * TK, TK), pl.ds(g0, LANES)], wq)

        total = HU * nc
        ss = {t: spre_ref[t] for t in range(LA)}
        acc = l = None
        nxt = None
        for t in range(total):
            j, c = divmod(t, nc)
            h0 = _mult((hg * HU + j) * DH, DH)
            if c == 0:
                acc = jnp.zeros((DH, TQ), _F32)
                l = jnp.zeros((8, TQ), _F32)
            if t + LA < total:
                ss[t + LA] = qk(t + LA)
            else:
                if nxt is None:
                    nxt = masked_q(hg_n * HU, q0_n)
                cn = t + LA - total
                spre_ref[cn] = _dot(k_ref[pl.ds(cn * TK, TK), pl.ds(nxt[1], LANES)], nxt[0])
            p = jnp.exp2(ss.pop(t))
            l = l + jnp.sum(p.reshape(TK // 8, 8, TQ), axis=0)
            acc = acc + _dot(vt_ref[pl.ds(h0, DH), pl.ds(c * TK, TK)], p.astype(_BF16))
            if c == nc - 1:
                lsum = jnp.sum(l, axis=0, keepdims=True)
                ot_ref[pl.ds(h0, DH), pl.ds(q0, TQ)] = (acc / lsum).astype(_BF16)

    for c, sv in enumerate(prefetch_qk(0, 0)):
        spre_ref[c] = sv

    def qblock(qb, carry):
        q0 = pl.multiple_of(qb * TQ, TQ)

        @pl.when(safe)
        def _fast():
            def body(hg, c):
                last = hg == nhg - 1
                hg_n = jnp.where(last, 0, hg + 1)
                qb_n = jnp.where(last, jnp.minimum(qb + 1, nq - 1), qb)
                fast_heads(hg, q0, hg_n, pl.multiple_of(qb_n * TQ, TQ))
                return c
            jax.lax.fori_loop(0, nhg, body, 0)

        @pl.when(jnp.logical_not(safe))
        def _slow():
            def body(h, c):
                h0 = pl.multiple_of(h * DH, DH)
                wq, g0 = masked_q(h, q0)
                s = _dot(k_ref[:, pl.ds(g0, LANES)], wq)
                m = jnp.max(s, axis=0, keepdims=True)
                p = jnp.exp2(s - m)
                lsum = jnp.sum(p, axis=0, keepdims=True)
                acc = _dot(vt_ref[pl.ds(h0, DH), :], p.astype(_BF16))
                ot_ref[pl.ds(h0, DH), pl.ds(q0, TQ)] = (acc / lsum).astype(_BF16)
                return c

            jax.lax.fori_loop(0, H, body, 0)

        finalize(qb)
        return carry

    jax.lax.fori_loop(0, nq, qblock, 0)

    for qb in range(nq):
        out_copy(qb).wait()


@jax.jit
def pallas_gated_mix__mha_block__mixer_s_mlp__prompt_kernel(
    A_x: jax.Array,
    A_wqkv: jax.Array,
    A_wo: jax.Array,
    B_x: jax.Array,
    B_w1: jax.Array,
    B_w2: jax.Array,
    B_w3: jax.Array,
    B_w4: jax.Array,
    gate_w: jax.Array,
):
    ax = A_x.reshape(S, D)
    hbm = pl.BlockSpec(memory_space=pl.ANY)
    out = pl.pallas_call(
        _kernel,
        out_shape=jax.ShapeDtypeStruct((S, D), A_x.dtype),
        in_specs=[hbm] * 8,
        out_specs=hbm,
        scratch_shapes=[
            pltpu.VMEM((S, D), _BF16),
            pltpu.VMEM((D, 3 * D), _BF16),
            pltpu.VMEM((D, D), _BF16),
            pltpu.VMEM((D, D), _BF16),
            pltpu.VMEM((D, D), _BF16),
            pltpu.VMEM((D, F), _BF16),
            pltpu.VMEM((F, D), _BF16),
            pltpu.VMEM((D,), _BF16),
            pltpu.VMEM((D, S), _BF16),
            pltpu.VMEM((S, D), _BF16),
            pltpu.VMEM((D, S), _BF16),
            pltpu.VMEM((D, S), _BF16),
            pltpu.VMEM((S + 2 * PAD, D), _F32),
            pltpu.VMEM((S, D), _F32),
            pltpu.VMEM((S, D), _BF16),
            pltpu.VMEM((3, H, RB), _F32),
            pltpu.VMEM((2 * D, D), _BF16),
            pltpu.VMEM((LA, TK, TQ), _F32),
            pltpu.SemaphoreType.DMA((NRB,)),
            pltpu.SemaphoreType.DMA((9,)),
            pltpu.SemaphoreType.DMA((S // TQ,)),
        ],
        compiler_params=pltpu.CompilerParams(vmem_limit_bytes=100 * 1024 * 1024),
    )(ax, A_wqkv, A_wo, B_w1, B_w2, B_w3, B_w4, gate_w)
    return out.reshape(1, S, D)
```

```python
import math

import jax
import jax.numpy as jnp
import jax.experimental.pallas as pl
import jax.experimental.pallas.tpu as pltpu

S = 2048
D = 512
H = 32
DH = 16
F = 1792
LANES = 128
HPG = LANES // DH
PAD = 8

TQ = 512
TK = 128
LA = 2
HU = 8
RB = 256
NRB = S // RB

LOG2E = math.log2(math.e)
QSCALE = (DH ** -0.5) * LOG2E
SAFE_LOG2 = 40.0
SAFE_V = 2.0 ** 60

_F32 = jnp.float32
_BF16 = jnp.bfloat16


def _dot(a, b):
    return jnp.dot(a, b, preferred_element_type=_F32)


def _dot_dims(a, b, ca, cb):
    return jax.lax.dot_general(a, b, (((ca,), (cb,)), ((), ())), preferred_element_type=_F32)


def _layernorm(x):
    m = jnp.mean(x, axis=-1, keepdims=True)
    xc = x - m
    v = jnp.mean(xc * xc, axis=-1, keepdims=True)
    return xc * jax.lax.rsqrt(v + 1e-5)


def _gelu(x):
    c = math.sqrt(2.0 / math.pi)
    return 0.5 * x * (1.0 + jnp.tanh(c * (x + 0.044715 * (x * x * x))))


def _mult(v, m):
    return v if isinstance(v, int) else pl.multiple_of(v, m)


def _kernel(x_hbm, wqkv_hbm, wo_hbm, w1_hbm, w2_hbm, w3_hbm, w4_hbm, gw_hbm,
            out_hbm,
            x_ref, wqkv_ref, wo_ref, w1_ref, w2_ref, w3_ref, w4_ref, gw_ref,
            qt_ref, k_ref, vt_ref, ot_ref, h_ref, b_ref, o_stage, nrm_ref, wqvt_ref, spre_ref,
            x_sems, w_sems, out_sems):
    def x_copy(r):
        r0 = _mult(r * RB, RB)
        return pltpu.make_async_copy(x_hbm.at[pl.ds(r0, RB), :], x_ref.at[pl.ds(r0, RB), :], x_sems.at[r])

    w_copies = {
        "wk": pltpu.make_async_copy(wqkv_hbm.at[:, pl.ds(D, D)], wqkv_ref.at[:, pl.ds(D, D)], w_sems.at[0]),
        "wq": pltpu.make_async_copy(wqkv_hbm.at[:, pl.ds(0, D)], wqkv_ref.at[:, pl.ds(0, D)], w_sems.at[1]),
        "wv": pltpu.make_async_copy(wqkv_hbm.at[:, pl.ds(2 * D, D)], wqkv_ref.at[:, pl.ds(2 * D, D)], w_sems.at[2]),
        "w1": pltpu.make_async_copy(w1_hbm, w1_ref, w_sems.at[3]),
        "w2": pltpu.make_async_copy(w2_hbm, w2_ref, w_sems.at[4]),
        "w3": pltpu.make_async_copy(w3_hbm, w3_ref, w_sems.at[5]),
        "w4": pltpu.make_async_copy(w4_hbm, w4_ref, w_sems.at[6]),
        "wo": pltpu.make_async_copy(wo_hbm, wo_ref, w_sems.at[7]),
        "gw": pltpu.make_async_copy(gw_hbm, gw_ref, w_sems.at[8]),
    }
    x_copy(0).start()
    for name in ("wk", "w1", "wq", "wv"):
        w_copies[name].start()
    for r in range(1, NRB):
        x_copy(r).start()
    for name in ("w2", "w3", "w4", "wo", "gw"):
        w_copies[name].start()

    head_of_col = jax.lax.broadcasted_iota(jnp.int32, (H, D), 1) // DH
    rowi = jax.lax.broadcasted_iota(jnp.int32, (H, D), 0)

    h_ref[pl.ds(0, PAD), :] = jnp.zeros((PAD, D), _F32)
    h_ref[pl.ds(PAD + S, PAD), :] = jnp.zeros((PAD, D), _F32)
    nrm_ref[...] = jnp.zeros(nrm_ref.shape, _F32)

    def proj(r, first):
        r0 = _mult(r * RB, RB)
        et_mat = jnp.where(head_of_col == rowi, 1.0, 0.0).astype(_BF16)
        x_copy(r).wait()
        x = x_ref[pl.ds(r0, RB), :]
        if first:
            w_copies["wk"].wait()
        kk = _dot(x, wqkv_ref[:, D:2 * D]).astype(_BF16)
        k_ref[pl.ds(r0, RB), :] = kk
        kf = kk.astype(_F32)
        kn = _dot_dims(et_mat, (kf * kf).astype(_BF16), 1, 1)
        if first:
            w_copies["w1"].wait()
        hh = _gelu(_dot(_layernorm(x.astype(_F32)).astype(_BF16), w1_ref[...]))
        h_ref[pl.ds(_mult(PAD + r0, 8), RB), :] = hh
        if first:
            w_copies["wq"].wait()
            w_copies["wv"].wait()
            wqvt_ref[pl.ds(0, D), :] = wqkv_ref[:, 0:D].T
            wqvt_ref[pl.ds(D, D), :] = wqkv_ref[:, 2 * D:3 * D].T
        qvt = _dot_dims(wqvt_ref[...], x, 1, 1)
        qt = (qvt[:D] * QSCALE).astype(_BF16)
        qt_ref[:, pl.ds(r0, RB)] = qt
        qf = qt.astype(_F32)
        qn = _dot(et_mat, (qf * qf).astype(_BF16))
        vt = qvt[D:].astype(_BF16)
        vt_ref[:, pl.ds(r0, RB)] = vt
        va = jnp.abs(vt.astype(_F32))
        vm = jnp.max(va.reshape(D // H, H, RB), axis=0)
        nrm_ref[0] = jnp.maximum(nrm_ref[0], qn)
        nrm_ref[1] = jnp.maximum(nrm_ref[1], kn)
        nrm_ref[2] = jnp.maximum(nrm_ref[2], vm)

    proj(0, True)

    def proj_body(r, c):
        proj(r, False)
        return c
    jax.lax.fori_loop(1, NRB, proj_body, 0)

    bound2 = jnp.max(nrm_ref[0]) * jnp.max(nrm_ref[1]) * 1.02
    safe = jnp.logical_and(bound2 <= SAFE_LOG2 * SAFE_LOG2, jnp.max(nrm_ref[2]) <= SAFE_V)

    for name in ("w2", "w3", "w4", "wo", "gw"):
        w_copies[name].wait()
    shifts = (-1, 1, -2, 2)

    def mlp_body(i, c):
        r0s = [pl.multiple_of((2 * i + u) * RB, RB) for u in range(2)]
        x1s = []
        for r0 in r0s:
            win = [h_ref[pl.ds(r0, RB + 2 * PAD), pl.ds(j * LANES, LANES)] for j in range(4)]
            hs_in = jnp.concatenate(
                [win[j][PAD + shifts[j]:PAD + shifts[j] + RB] for j in range(4)], axis=-1).astype(_BF16)
            x1s.append(x_ref[pl.ds(r0, RB), :].astype(_F32) + _dot(hs_in, w2_ref[...]))
        h2s = [_gelu(_dot(_layernorm(x1).astype(_BF16), w3_ref[...])).astype(_BF16) for x1 in x1s]
        for r0, x1, h2 in zip(r0s, x1s, h2s):
            b_ref[pl.ds(r0, RB), :] = x1 + _dot(h2, w4_ref[...])
        return c
    jax.lax.fori_loop(0, NRB // 2, mlp_body, 0)

    nq = S // TQ
    nc = S // TK

    def masked_q(h, q0):
        g0 = _mult((h // HPG) * LANES, LANES)
        qg = qt_ref[pl.ds(g0, LANES), pl.ds(q0, TQ)]
        row = jax.lax.broadcasted_iota(jnp.int32, (LANES, TQ), 0) // DH
        return jnp.where(row == (h % HPG), qg, jnp.zeros_like(qg)), g0

    def out_copy(r):
        r0 = _mult(r * RB, RB)
        return pltpu.make_async_copy(o_stage.at[pl.ds(r0, RB), :], out_hbm.at[pl.ds(r0, RB), :], out_sems.at[r])

    def finalize(qb):
        for r in range(TQ // RB):
            rb = qb * (TQ // RB) + r
            r0 = pl.multiple_of(rb * RB, RB)
            a = _dot_dims(ot_ref[:, pl.ds(r0, RB)], wo_ref[...], 0, 0)
            xa = x_ref[pl.ds(r0, RB), :].astype(_F32)
            g = jax.nn.sigmoid(jnp.sum(xa * gw_ref[...].astype(_F32).reshape(1, D), axis=-1, keepdims=True))
            o_stage[pl.ds(r0, RB), :] = (g * a + (1.0 - g) * b_ref[pl.ds(r0, RB), :]).astype(o_stage.dtype)
            out_copy(rb).start()

    nhg = H // HU

    def prefetch_qk(hg, q0):
        wq, g0 = masked_q(hg * HU, q0)
        return [_dot(k_ref[pl.ds(c * TK, TK), pl.ds(g0, LANES)], wq) for c in range(LA)]

    def fast_heads(hg, q0, hg_n, q0_n):
        wqs = {}

        def qk(t):
            j, c = divmod(t, nc)
            if j not in wqs:
                wqs[j] = masked_q(hg * HU + j, q0)
            wq, g0 = wqs[j]
            return _dot(k_ref[pl.ds(c * TK, TK), pl.ds(g0, LANES)], wq)

        total = HU * nc
        ss = {t: spre_ref[t] for t in range(LA)}
        acc = l = None
        nxt = None
        for t in range(total):
            j, c = divmod(t, nc)
            h0 = _mult((hg * HU + j) * DH, DH)
            if c == 0:
                acc = jnp.zeros((DH, TQ), _F32)
                l = jnp.zeros((8, TQ), _F32)
            if t + LA < total:
                ss[t + LA] = qk(t + LA)
            else:
                if nxt is None:
                    nxt = masked_q(hg_n * HU, q0_n)
                cn = t + LA - total
                spre_ref[cn] = _dot(k_ref[pl.ds(cn * TK, TK), pl.ds(nxt[1], LANES)], nxt[0])
            p = jnp.exp2(ss.pop(t))
            l = l + jnp.sum(p.reshape(TK // 8, 8, TQ), axis=0)
            acc = acc + _dot(vt_ref[pl.ds(h0, DH), pl.ds(c * TK, TK)], p.astype(_BF16))
            if c == nc - 1:
                lsum = jnp.sum(l, axis=0, keepdims=True)
                ot_ref[pl.ds(h0, DH), pl.ds(q0, TQ)] = (acc / lsum).astype(_BF16)

    for c, sv in enumerate(prefetch_qk(0, 0)):
        spre_ref[c] = sv

    def qblock(qb, carry):
        q0 = pl.multiple_of(qb * TQ, TQ)

        @pl.when(safe)
        def _fast():
            def body(hg, c):
                last = hg == nhg - 1
                hg_n = jnp.where(last, 0, hg + 1)
                qb_n = jnp.where(last, jnp.minimum(qb + 1, nq - 1), qb)
                fast_heads(hg, q0, hg_n, pl.multiple_of(qb_n * TQ, TQ))
                return c
            jax.lax.fori_loop(0, nhg, body, 0)

        @pl.when(jnp.logical_not(safe))
        def _slow():
            def body(h, c):
                h0 = pl.multiple_of(h * DH, DH)
                wq, g0 = masked_q(h, q0)
                s = _dot(k_ref[:, pl.ds(g0, LANES)], wq)
                m = jnp.max(s, axis=0, keepdims=True)
                p = jnp.exp2(s - m)
                lsum = jnp.sum(p, axis=0, keepdims=True)
                acc = _dot(vt_ref[pl.ds(h0, DH), :], p.astype(_BF16))
                ot_ref[pl.ds(h0, DH), pl.ds(q0, TQ)] = (acc / lsum).astype(_BF16)
                return c

            jax.lax.fori_loop(0, H, body, 0)

        finalize(qb)
        return carry

    jax.lax.fori_loop(0, nq, qblock, 0)

    for r in range(NRB):
        out_copy(r).wait()


@jax.jit
def pallas_gated_mix__mha_block__mixer_s_mlp__prompt_kernel(
    A_x: jax.Array,
    A_wqkv: jax.Array,
    A_wo: jax.Array,
    B_x: jax.Array,
    B_w1: jax.Array,
    B_w2: jax.Array,
    B_w3: jax.Array,
    B_w4: jax.Array,
    gate_w: jax.Array,
):
    ax = A_x.reshape(S, D)
    hbm = pl.BlockSpec(memory_space=pl.ANY)
    out = pl.pallas_call(
        _kernel,
        out_shape=jax.ShapeDtypeStruct((S, D), A_x.dtype),
        in_specs=[hbm] * 8,
        out_specs=hbm,
        scratch_shapes=[
            pltpu.VMEM((S, D), _BF16),
            pltpu.VMEM((D, 3 * D), _BF16),
            pltpu.VMEM((D, D), _BF16),
            pltpu.VMEM((D, D), _BF16),
            pltpu.VMEM((D, D), _BF16),
            pltpu.VMEM((D, F), _BF16),
            pltpu.VMEM((F, D), _BF16),
            pltpu.VMEM((D,), _BF16),
            pltpu.VMEM((D, S), _BF16),
            pltpu.VMEM((S, D), _BF16),
            pltpu.VMEM((D, S), _BF16),
            pltpu.VMEM((D, S), _BF16),
            pltpu.VMEM((S + 2 * PAD, D), _F32),
            pltpu.VMEM((S, D), _F32),
            pltpu.VMEM((S, D), _BF16),
            pltpu.VMEM((3, H, RB), _F32),
            pltpu.VMEM((2 * D, D), _BF16),
            pltpu.VMEM((LA, TK, TQ), _F32),
            pltpu.SemaphoreType.DMA((NRB,)),
            pltpu.SemaphoreType.DMA((9,)),
            pltpu.SemaphoreType.DMA((NRB,)),
        ],
        compiler_params=pltpu.CompilerParams(vmem_limit_bytes=100 * 1024 * 1024),
    )(ax, A_wqkv, A_wo, B_w1, B_w2, B_w3, B_w4, gate_w)
    return out.reshape(1, S, D)
```

```python
import math

import jax
import jax.numpy as jnp
import jax.experimental.pallas as pl
import jax.experimental.pallas.tpu as pltpu

S = 2048
D = 512
H = 32
DH = 16
F = 1792
LANES = 128
HPG = LANES // DH
PAD = 8

TQ = 512
TK = 128
LA = 2
HU = 8
RB = 256
NRB = S // RB

LOG2E = math.log2(math.e)
QSCALE = (DH ** -0.5) * LOG2E
SAFE_LOG2 = 40.0
SAFE_V = 2.0 ** 60

_F32 = jnp.float32
_BF16 = jnp.bfloat16


def _dot(a, b):
    return jnp.dot(a, b, preferred_element_type=_F32)


def _dot_dims(a, b, ca, cb):
    return jax.lax.dot_general(a, b, (((ca,), (cb,)), ((), ())), preferred_element_type=_F32)


def _layernorm(x):
    m = jnp.mean(x, axis=-1, keepdims=True)
    xc = x - m
    v = jnp.mean(xc * xc, axis=-1, keepdims=True)
    return xc * jax.lax.rsqrt(v + 1e-5)


def _gelu(x):
    c = math.sqrt(2.0 / math.pi)
    return 0.5 * x * (1.0 + jnp.tanh(c * (x + 0.044715 * (x * x * x))))


def _mult(v, m):
    return v if isinstance(v, int) else pl.multiple_of(v, m)


def _kernel(x_hbm, wqkv_hbm, wo_hbm, w1_hbm, w2_hbm, w3_hbm, w4_hbm, gw_hbm,
            out_hbm,
            x_ref, wqkv_ref, wo_ref, w1_ref, w2_ref, w3_ref, w4_ref, gw_ref,
            qt_ref, k_ref, vt_ref, ot_ref, h_ref, b_ref, o_stage, nrm_ref, wqvt_ref, spre_ref,
            x_sems, w_sems, out_sems):
    def x_copy(r):
        r0 = _mult(r * RB, RB)
        return pltpu.make_async_copy(x_hbm.at[pl.ds(r0, RB), :], x_ref.at[pl.ds(r0, RB), :], x_sems.at[r])

    w_copies = {
        "wk": pltpu.make_async_copy(wqkv_hbm.at[:, pl.ds(D, D)], wqkv_ref.at[:, pl.ds(D, D)], w_sems.at[0]),
        "wq": pltpu.make_async_copy(wqkv_hbm.at[:, pl.ds(0, D)], wqkv_ref.at[:, pl.ds(0, D)], w_sems.at[1]),
        "wv": pltpu.make_async_copy(wqkv_hbm.at[:, pl.ds(2 * D, D)], wqkv_ref.at[:, pl.ds(2 * D, D)], w_sems.at[2]),
        "w1": pltpu.make_async_copy(w1_hbm, w1_ref, w_sems.at[3]),
        "w2": pltpu.make_async_copy(w2_hbm, w2_ref, w_sems.at[4]),
        "w3": pltpu.make_async_copy(w3_hbm, w3_ref, w_sems.at[5]),
        "w4": pltpu.make_async_copy(w4_hbm, w4_ref, w_sems.at[6]),
        "wo": pltpu.make_async_copy(wo_hbm, wo_ref, w_sems.at[7]),
        "gw": pltpu.make_async_copy(gw_hbm, gw_ref, w_sems.at[8]),
    }
    x_copy(0).start()
    for name in ("wk", "w1"):
        w_copies[name].start()
    x_copy(1).start()
    for name in ("wq", "wv"):
        w_copies[name].start()
    for r in range(2, NRB):
        x_copy(r).start()
    for name in ("w2", "w3", "w4", "wo", "gw"):
        w_copies[name].start()

    head_of_col = jax.lax.broadcasted_iota(jnp.int32, (H, D), 1) // DH
    rowi = jax.lax.broadcasted_iota(jnp.int32, (H, D), 0)

    h_ref[pl.ds(0, PAD), :] = jnp.zeros((PAD, D), _F32)
    h_ref[pl.ds(PAD + S, PAD), :] = jnp.zeros((PAD, D), _F32)
    nrm_ref[...] = jnp.zeros(nrm_ref.shape, _F32)

    def et_matrix():
        return jnp.where(head_of_col == rowi, 1.0, 0.0).astype(_BF16)

    def proj_k(r):
        r0 = _mult(r * RB, RB)
        x = x_ref[pl.ds(r0, RB), :]
        kk = _dot(x, wqkv_ref[:, D:2 * D]).astype(_BF16)
        k_ref[pl.ds(r0, RB), :] = kk
        kf = kk.astype(_F32)
        kn = _dot_dims(et_matrix(), (kf * kf).astype(_BF16), 1, 1)
        nrm_ref[1] = jnp.maximum(nrm_ref[1], kn)

    def proj_h(r):
        r0 = _mult(r * RB, RB)
        x = x_ref[pl.ds(r0, RB), :]
        hh = _gelu(_dot(_layernorm(x.astype(_F32)).astype(_BF16), w1_ref[...]))
        h_ref[pl.ds(_mult(PAD + r0, 8), RB), :] = hh

    def proj_qv(r):
        r0 = _mult(r * RB, RB)
        x = x_ref[pl.ds(r0, RB), :]
        qvt = _dot_dims(wqvt_ref[...], x, 1, 1)
        qt = (qvt[:D] * QSCALE).astype(_BF16)
        qt_ref[:, pl.ds(r0, RB)] = qt
        qf = qt.astype(_F32)
        qn = _dot(et_matrix(), (qf * qf).astype(_BF16))
        vt = qvt[D:].astype(_BF16)
        vt_ref[:, pl.ds(r0, RB)] = vt
        va = jnp.abs(vt.astype(_F32))
        vm = jnp.max(va.reshape(D // H, H, RB), axis=0)
        nrm_ref[0] = jnp.maximum(nrm_ref[0], qn)
        nrm_ref[2] = jnp.maximum(nrm_ref[2], vm)

    x_copy(0).wait()
    w_copies["wk"].wait()
    proj_k(0)
    w_copies["w1"].wait()
    x_copy(1).wait()
    proj_h(0)
    proj_k(1)
    proj_h(1)
    w_copies["wq"].wait()
    w_copies["wv"].wait()
    wqvt_ref[pl.ds(0, D), :] = wqkv_ref[:, 0:D].T
    wqvt_ref[pl.ds(D, D), :] = wqkv_ref[:, 2 * D:3 * D].T
    proj_qv(0)
    proj_qv(1)

    def proj_body(r, c):
        x_copy(r).wait()
        proj_k(r)
        proj_h(r)
        proj_qv(r)
        return c
    jax.lax.fori_loop(2, NRB, proj_body, 0)

    bound2 = jnp.max(nrm_ref[0]) * jnp.max(nrm_ref[1]) * 1.02
    safe = jnp.logical_and(bound2 <= SAFE_LOG2 * SAFE_LOG2, jnp.max(nrm_ref[2]) <= SAFE_V)

    for name in ("w2", "w3", "w4", "wo", "gw"):
        w_copies[name].wait()
    shifts = (-1, 1, -2, 2)

    def mlp_body(i, c):
        r0s = [pl.multiple_of((2 * i + u) * RB, RB) for u in range(2)]
        x1s = []
        for r0 in r0s:
            win = [h_ref[pl.ds(r0, RB + 2 * PAD), pl.ds(j * LANES, LANES)] for j in range(4)]
            hs_in = jnp.concatenate(
                [win[j][PAD + shifts[j]:PAD + shifts[j] + RB] for j in range(4)], axis=-1).astype(_BF16)
            x1s.append(x_ref[pl.ds(r0, RB), :].astype(_F32) + _dot(hs_in, w2_ref[...]))
        h2s = [_gelu(_dot(_layernorm(x1).astype(_BF16), w3_ref[...])).astype(_BF16) for x1 in x1s]
        for r0, x1, h2 in zip(r0s, x1s, h2s):
            b_ref[pl.ds(r0, RB), :] = x1 + _dot(h2, w4_ref[...])
        return c
    jax.lax.fori_loop(0, NRB // 2, mlp_body, 0)

    nq = S // TQ
    nc = S // TK

    def masked_q(h, q0):
        g0 = _mult((h // HPG) * LANES, LANES)
        qg = qt_ref[pl.ds(g0, LANES), pl.ds(q0, TQ)]
        row = jax.lax.broadcasted_iota(jnp.int32, (LANES, TQ), 0) // DH
        return jnp.where(row == (h % HPG), qg, jnp.zeros_like(qg)), g0

    def out_copy(r):
        r0 = _mult(r * RB, RB)
        return pltpu.make_async_copy(o_stage.at[pl.ds(r0, RB), :], out_hbm.at[pl.ds(r0, RB), :], out_sems.at[r])

    def finalize(qb):
        for r in range(TQ // RB):
            rb = qb * (TQ // RB) + r
            r0 = pl.multiple_of(rb * RB, RB)
            a = _dot_dims(ot_ref[:, pl.ds(r0, RB)], wo_ref[...], 0, 0)
            xa = x_ref[pl.ds(r0, RB), :].astype(_F32)
            g = jax.nn.sigmoid(jnp.sum(xa * gw_ref[...].astype(_F32).reshape(1, D), axis=-1, keepdims=True))
            o_stage[pl.ds(r0, RB), :] = (g * a + (1.0 - g) * b_ref[pl.ds(r0, RB), :]).astype(o_stage.dtype)
            out_copy(rb).start()

    nhg = H // HU

    def prefetch_qk(hg, q0):
        wq, g0 = masked_q(hg * HU, q0)
        return [_dot(k_ref[pl.ds(c * TK, TK), pl.ds(g0, LANES)], wq) for c in range(LA)]

    def fast_heads(hg, q0, hg_n, q0_n):
        wqs = {}

        def qk(t):
            j, c = divmod(t, nc)
            if j not in wqs:
                wqs[j] = masked_q(hg * HU + j, q0)
            wq, g0 = wqs[j]
            return _dot(k_ref[pl.ds(c * TK, TK), pl.ds(g0, LANES)], wq)

        total = HU * nc
        ss = {t: spre_ref[t] for t in range(LA)}
        acc = l = None
        nxt = None
        for t in range(total):
            j, c = divmod(t, nc)
            h0 = _mult((hg * HU + j) * DH, DH)
            if c == 0:
                acc = jnp.zeros((DH, TQ), _F32)
                l = jnp.zeros((8, TQ), _F32)
            if t + LA < total:
                ss[t + LA] = qk(t + LA)
            else:
                if nxt is None:
                    nxt = masked_q(hg_n * HU, q0_n)
                cn = t + LA - total
                spre_ref[cn] = _dot(k_ref[pl.ds(cn * TK, TK), pl.ds(nxt[1], LANES)], nxt[0])
            p = jnp.exp2(ss.pop(t))
            l = l + jnp.sum(p.reshape(TK // 8, 8, TQ), axis=0)
            acc = acc + _dot(vt_ref[pl.ds(h0, DH), pl.ds(c * TK, TK)], p.astype(_BF16))
            if c == nc - 1:
                lsum = jnp.sum(l, axis=0, keepdims=True)
                ot_ref[pl.ds(h0, DH), pl.ds(q0, TQ)] = (acc / lsum).astype(_BF16)

    for c, sv in enumerate(prefetch_qk(0, 0)):
        spre_ref[c] = sv

    def qblock(qb, carry):
        q0 = pl.multiple_of(qb * TQ, TQ)

        @pl.when(safe)
        def _fast():
            def body(hg, c):
                last = hg == nhg - 1
                hg_n = jnp.where(last, 0, hg + 1)
                qb_n = jnp.where(last, jnp.minimum(qb + 1, nq - 1), qb)
                fast_heads(hg, q0, hg_n, pl.multiple_of(qb_n * TQ, TQ))
                return c
            jax.lax.fori_loop(0, nhg, body, 0)

        @pl.when(jnp.logical_not(safe))
        def _slow():
            def body(h, c):
                h0 = pl.multiple_of(h * DH, DH)
                wq, g0 = masked_q(h, q0)
                s = _dot(k_ref[:, pl.ds(g0, LANES)], wq)
                m = jnp.max(s, axis=0, keepdims=True)
                p = jnp.exp2(s - m)
                lsum = jnp.sum(p, axis=0, keepdims=True)
                acc = _dot(vt_ref[pl.ds(h0, DH), :], p.astype(_BF16))
                ot_ref[pl.ds(h0, DH), pl.ds(q0, TQ)] = (acc / lsum).astype(_BF16)
                return c

            jax.lax.fori_loop(0, H, body, 0)

        finalize(qb)
        return carry

    jax.lax.fori_loop(0, nq, qblock, 0)

    for r in range(NRB):
        out_copy(r).wait()


@jax.jit
def pallas_gated_mix__mha_block__mixer_s_mlp__prompt_kernel(
    A_x: jax.Array,
    A_wqkv: jax.Array,
    A_wo: jax.Array,
    B_x: jax.Array,
    B_w1: jax.Array,
    B_w2: jax.Array,
    B_w3: jax.Array,
    B_w4: jax.Array,
    gate_w: jax.Array,
):
    ax = A_x.reshape(S, D)
    hbm = pl.BlockSpec(memory_space=pl.ANY)
    out = pl.pallas_call(
        _kernel,
        out_shape=jax.ShapeDtypeStruct((S, D), A_x.dtype),
        in_specs=[hbm] * 8,
        out_specs=hbm,
        scratch_shapes=[
            pltpu.VMEM((S, D), _BF16),
            pltpu.VMEM((D, 3 * D), _BF16),
            pltpu.VMEM((D, D), _BF16),
            pltpu.VMEM((D, D), _BF16),
            pltpu.VMEM((D, D), _BF16),
            pltpu.VMEM((D, F), _BF16),
            pltpu.VMEM((F, D), _BF16),
            pltpu.VMEM((D,), _BF16),
            pltpu.VMEM((D, S), _BF16),
            pltpu.VMEM((S, D), _BF16),
            pltpu.VMEM((D, S), _BF16),
            pltpu.VMEM((D, S), _BF16),
            pltpu.VMEM((S + 2 * PAD, D), _F32),
            pltpu.VMEM((S, D), _F32),
            pltpu.VMEM((S, D), _BF16),
            pltpu.VMEM((3, H, RB), _F32),
            pltpu.VMEM((2 * D, D), _BF16),
            pltpu.VMEM((LA, TK, TQ), _F32),
            pltpu.SemaphoreType.DMA((NRB,)),
            pltpu.SemaphoreType.DMA((9,)),
            pltpu.SemaphoreType.DMA((NRB,)),
        ],
        compiler_params=pltpu.CompilerParams(vmem_limit_bytes=100 * 1024 * 1024),
    )(ax, A_wqkv, A_wo, B_w1, B_w2, B_w3, B_w4, gate_w)
    return out.reshape(1, S, D)
```
